```python
import os as _os
_os.environ.setdefault("JAX_PLATFORMS", "cpu")
import jax
import jax.numpy as jnp

def _softmax(x, axis=-1):
    return jax.nn.softmax(x, axis=axis)
def _gelu(x):
    return jax.nn.gelu(x, approximate=True)
def _silu(x):
    return jax.nn.silu(x)
def _sigmoid(x):
    return jax.nn.sigmoid(x)
def _layernorm(x, axis=-1, eps=1e-5):
    m = jnp.mean(x, axis=axis, keepdims=True)
    v = jnp.var(x, axis=axis, keepdims=True)
    return (x - m) / jnp.sqrt(v + eps)
def _scatter_add(tgt, idx, src, axis=0):
    return tgt.at[idx].add(src)
def _segment_sum(src, seg, n):
    return jax.ops.segment_sum(src, seg, n)
class _Rng:
    def __init__(self, key):
        self._k = key
    def _next(self):
        self._k, sub = jax.random.split(self._k)
        return sub
    def normal(self, shape):
        return jax.random.normal(self._next(), shape, dtype=jnp.bfloat16)
    def randint(self, lo, hi, shape):
        return jax.random.randint(self._next(), shape, lo, hi, dtype=jnp.int32)
    def uniform(self, shape, lo=0.0, hi=1.0):
        return jax.random.uniform(self._next(), shape, jnp.bfloat16, lo, hi)
    def permutation(self, n):
        return jax.random.permutation(self._next(), n)


kernel_name = 'standalone__detection_seg_fpn_lateral__vision'

def setup_inputs():
    _rng = _Rng(jax.random.key(int.from_bytes(__import__("os").urandom(4), "little")))
    _w = (lambda a: (lambda t: t.astype(jnp.bfloat16) if jnp.issubdtype(t.dtype, jnp.floating) else t)(jnp.asarray(a)))
    H = W = (256 // 2) * 2
    C = 384
    k = 1
    return {
        "c_fine": _w((lambda *s: _rng.normal(s) * 0.05)(1, H, W, C)),
        "p_coarse": _w((lambda *s: _rng.normal(s) * 0.05)(1, H // 2, W // 2, C)),
        "w_lat": _w((lambda *s: _rng.normal(s) * 0.05)(C, C)),
        "w_out": _w((lambda *s: _rng.normal(s) * 0.05)(k, k, C, C)),
    }

def reference(c_fine, p_coarse, w_lat, w_out):
    B, H, W, C = c_fine.shape
    k = 1
    lat = jnp.einsum("bhwc,cd->bhwd", c_fine, w_lat)
    up = jnp.repeat(jnp.repeat(p_coarse, 2, axis=1), 2, axis=2)
    m = lat + up
    pad = k // 2
    mp = jnp.pad(m, ((0, 0), (pad, pad), (pad, pad), (0, 0)))
    o = None
    for di in range(k):
        for dj in range(k):
            t = jnp.einsum("bhwc,cd->bhwd", mp[:, di:di + H, dj:dj + W, :], w_out[di, dj])
            o = t if o is None else o + t
    return o
```

```python
import jax
import jax.numpy as jnp
from jax import lax
import jax.experimental.pallas as pl
import jax.experimental.pallas.tpu as pltpu

_A = 16
_S = 32
_SWITCH = 37
_BACKLOG = 4
_RATE = 2


@jax.jit
def pallas_standalone__detection_seg_fpn_lateral__vision_kernel(
    c_fine: jax.Array,
    p_coarse: jax.Array,
    w_lat: jax.Array,
    w_out: jax.Array,
):
    B, H, W, C = c_fine.shape
    A, S = _A, _S
    I = B * H // 2 // A
    NW = W // S
    NU = I * NW
    S2 = S // 2
    NL = C // 128
    dtype = c_fine.dtype

    chunks, u = [], 0
    while u < NW:
        n = min(max(u, 1), NW - u)
        chunks.append((u, n))
        u += n
    chunks += [(NW, NW // 2), (NW + NW // 2, NW // 2)]
    chunks += [(i * NW, NW) for i in range(2, I)]
    NCH = len(chunks)

    def kernel_function(c_hbm, p_hbm, wl_hbm, wo_hbm, o_hbm,
                        cb, pb, ob, wl, wo, wf, qs, rsem, wsem):
        def reads(k):
            u0, n = chunks[k]
            i0, w0 = divmod(u0, NW)
            if n >= NW:
                cs = [(slice(None), pl.ds(i0, n // NW))]
                ps = cs[0]
            else:
                cs = [(slice(None), i0, j, pl.ds(w0 * S, n * S)) for j in range(2)]
                ps = (slice(None), i0, pl.ds(w0 * S2, n * S2))
            return [pltpu.make_async_copy(p_hbm.at[ps], pb.at[ps], rsem.at[k])] + [
                pltpu.make_async_copy(c_hbm.at[s], cb.at[s], rsem.at[k]) for s in cs
            ]

        def write(u, carry):
            i = u // NW
            w0 = pl.multiple_of((u % NW) * S, S)
            for j in range(2):
                s = (slice(None), i, j, pl.ds(w0, S))
                pltpu.make_async_copy(ob.at[s], o_hbm.at[s], wsem.at[0]).start()
            return carry

        weights = [
            pltpu.make_async_copy(wl_hbm, wl, rsem.at[NCH]),
            pltpu.make_async_copy(wo_hbm, wo, rsem.at[NCH]),
        ]
        for x in weights:
            x.start()
        for k in range(NCH):
            for x in reads(k):
                x.start()
        for x in weights:
            x.wait()
        wf[...] = jnp.dot(
            wl[...], wo[...], preferred_element_type=jnp.float32
        ).astype(wf.dtype)

        def compute(u):
            i = u // NW
            wc = u % NW
            w0 = pl.multiple_of(wc * S, S)
            v0 = pl.multiple_of(wc * S2, S2)
            pv = pb[:, i, pl.ds(v0, S2), :].reshape(A * S2, C)
            q = jnp.dot(pv, wo[...], preferred_element_type=jnp.float32)
            for n in range(NL):
                for e in range(2):
                    qs[n, pl.ds(e, A * S2, stride=2), :] = q[:, n * 128:(n + 1) * 128]
            up = jnp.concatenate([qs[n] for n in range(NL)], axis=1)
            for j in range(2):
                cv = cb[:, i, j, pl.ds(w0, S), :].reshape(A * S, C)
                acc = jnp.dot(cv, wf[...], preferred_element_type=jnp.float32)
                ob[:, i, j, pl.ds(w0, S), :] = (acc + up).astype(dtype).reshape(A, S, C)

        def body(u, done):
            for k in range(NCH):
                @pl.when(u == min(chunks[k][0], _SWITCH))
                def _():
                    for x in reads(k):
                        x.wait()
            tgt = jnp.where(
                u >= _SWITCH, jnp.minimum(_BACKLOG + (u - _SWITCH) * _RATE, u), 0
            )
            lax.fori_loop(done, tgt, write, None)
            compute(u)
            return tgt

        done = lax.fori_loop(0, NU, body, 0)
        lax.fori_loop(done, NU, write, None)
        pltpu.make_async_copy(ob, o_hbm, wsem.at[0]).wait()

    out = pl.pallas_call(
        kernel_function,
        in_specs=[pl.BlockSpec(memory_space=pl.ANY)] * 4,
        out_specs=pl.BlockSpec(memory_space=pl.ANY),
        out_shape=jax.ShapeDtypeStruct((A, I, 2, W, C), dtype),
        scratch_shapes=[
            pltpu.VMEM((A, I, 2, W, C), dtype),
            pltpu.VMEM((A, I, W // 2, C), p_coarse.dtype),
            pltpu.VMEM((A, I, 2, W, C), dtype),
            pltpu.VMEM((C, C), w_lat.dtype),
            pltpu.VMEM((C, C), w_out.dtype),
            pltpu.VMEM((C, C), dtype),
            pltpu.VMEM((NL, A * S, 128), jnp.float32),
            pltpu.SemaphoreType.DMA((NCH + 1,)),
            pltpu.SemaphoreType.DMA((1,)),
        ],
        compiler_params=pltpu.CompilerParams(vmem_limit_bytes=124 * 2**20),
    )(
        c_fine.reshape(A, I, 2, W, C),
        p_coarse.reshape(A, I, W // 2, C),
        w_lat,
        w_out.reshape(C, C),
    )
    return out.reshape(B, H, W, C)
```

```python
import jax
import jax.numpy as jnp
from jax import lax
import jax.experimental.pallas as pl
import jax.experimental.pallas.tpu as pltpu

_LANES = 128
_STREAMS = 6
_PIECE = 32
_ROWS = 4
_READ_STEPS = 0.6
_LAST_READ = 3
_BATCH = 8
_BACKLOG = 40
_PACE = 22


@jax.jit
def pallas_standalone__detection_seg_fpn_lateral__vision_kernel(
    c_fine: jax.Array,
    p_coarse: jax.Array,
    w_lat: jax.Array,
    w_out: jax.Array,
):
    B, H, W, C = c_fine.shape
    dtype = c_fine.dtype
    A, S, G = _STREAMS, _PIECE, _ROWS
    n_rows = B * H // 2
    band = n_rows // A
    spare = n_rows - A * band
    ppr = 2 * W // S
    n_pieces = n_rows * ppr
    stream = n_pieces // A
    n_steps = n_rows // G
    n_tiles = C // _LANES
    assert w_out.shape == (1, 1, C, C) and p_coarse.shape == (B, H // 2, W // 2, C)
    assert n_rows % G == 0 and W % S == 0 and C % _LANES == 0
    assert 0 < spare < G and ppr % _BATCH == 0

    order = list(range(A * band, n_rows))
    order += [a * band + i for i in range(band) for a in reversed(range(A))]
    step_of = {row: pos // G for pos, row in enumerate(order)}
    switch = int(_READ_STEPS * n_steps)

    lead = G - spare
    chunks = [(A - lead, lead, 0, 1), (0, A - lead, 0, 1)]
    i = 1
    while i < band:
        n = min(max(i // 2, 1), band - i)
        chunks.append((0, A, i, n))
        i += n
    n_chunks = len(chunks)
    read_due = [min(step_of[(a + na - 1) * band + i], switch) for a, na, i, _ in chunks]
    last_read_due = step_of[A * band - 1]

    def ready(k):
        return max(step_of[(a * stream + k) // ppr] for a in range(A)) + 1

    early = range(band * ppr, stream)
    assert all(ready(k) <= switch for k in early)
    write_due = []
    for k in range(0, band * ppr, _BATCH):
        paced = switch + pl.cdiv(max(k + _BATCH - _BACKLOG, 0), _PACE)
        needs = [ready(k + b) for b in range(_BATCH)]
        write_due.append(max([min(paced, n_steps)] + needs + write_due[-1:]))

    def kernel_function(c_hbm, p_hbm, wl_hbm, wo_hbm, o_hbm,
                        c_buf, p_buf, o_buf, wl, wo, wf, up_buf, out_sem):
        def split(ref, n):
            return ref.at[pl.ds(0, A * n)].reshape(A, n, *ref.shape[1:])

        def copy(src, dst, idx, sem):
            return pltpu.make_async_copy(src.at[idx], dst.at[idx], sem)

        def write(k):
            copy(split(o_buf, stream), split(o_hbm, stream), (slice(None), k),
                 out_sem.at[0]).start()

        def write_batch(b, carry):
            for k in range(_BATCH):
                write(b * _BATCH + k)
            return carry

        def compute(step):
            rows = []
            for g in range(G):
                pos = step * G + g - spare
                banded = (A - 1 - lax.rem(pos, A)) * band + lax.div(pos, A)
                rows.append(jnp.where(pos < 0, n_rows + pos, banded))
            p = jnp.concatenate([p_buf[r] for r in rows], axis=0)
            q = jnp.dot(p, wo[...], preferred_element_type=jnp.float32)
            for t in range(n_tiles):
                for e in range(2):
                    up_buf[t, pl.ds(e, G * W // 2, stride=2), :] = (
                        q[:, t * _LANES:(t + 1) * _LANES])
            up = jnp.concatenate([up_buf[t] for t in range(n_tiles)], axis=1)
            for j in range(2):
                idx = [pl.ds(r * ppr + j * (W // S), W // S) for r in rows]
                c = jnp.concatenate([c_buf[s].reshape(W, C) for s in idx], axis=0)
                lat = jnp.dot(c, wf[...], preferred_element_type=jnp.float32)
                res = (lat + up).astype(dtype)
                for g, s in enumerate(idx):
                    o_buf[s] = res[g * W:(g + 1) * W].reshape(W // S, S, C)

        def run(in_sem):
            def weights():
                return [pltpu.make_async_copy(wl_hbm, wl, in_sem.at[n_chunks]),
                        pltpu.make_async_copy(wo_hbm, wo, in_sem.at[n_chunks])]

            def reads(k):
                a, na, i, n = chunks[k]
                held = _LAST_READ if k == n_chunks - 1 else 0
                sem = in_sem.at[k]
                copies = [
                    copy(split(p_hbm, band), split(p_buf, band),
                         (pl.ds(a, na), pl.ds(i, n)), sem),
                    copy(split(c_hbm, band * ppr), split(c_buf, band * ppr),
                         (pl.ds(a, na), pl.ds(i * ppr, n * ppr - held)), sem),
                ]
                if k == 0:
                    copies += [
                        copy(p_hbm, p_buf, pl.ds(A * band, spare), sem),
                        copy(c_hbm, c_buf, pl.ds(A * band * ppr, spare * ppr), sem),
                    ]
                return copies

            def last_read():
                return copy(split(c_hbm, band * ppr), split(c_buf, band * ppr),
                            (slice(None), pl.ds(band * ppr - _LAST_READ, _LAST_READ)),
                            in_sem.at[n_chunks + 1])

            for x in weights():
                x.start()
            for k in range(n_chunks):
                for x in reads(k):
                    x.start()
            last_read().start()

            for x in weights():
                x.wait()
            wf[...] = jnp.dot(
                wl[...], wo[...], preferred_element_type=jnp.float32
            ).astype(wf.dtype)

            def body(step, queued):
                for k in range(n_chunks):
                    @pl.when(step == read_due[k])
                    def _(k=k):
                        for x in reads(k):
                            x.wait()

                @pl.when(step == switch)
                def _():
                    for k in early:
                        write(k)
                    if A * stream < n_pieces:
                        copy(o_buf, o_hbm, pl.ds(A * stream, n_pieces - A * stream),
                             out_sem.at[0]).start()

                target = queued
                for due in sorted(set(write_due) - {n_steps}):
                    count = sum(d <= due for d in write_due)
                    target = jnp.where(step == due, count, target)
                lax.fori_loop(queued, target, write_batch, None)

                @pl.when(step == last_read_due)
                def _():
                    last_read().wait()

                compute(step)
                return target

            queued = lax.fori_loop(0, n_steps, body, 0)
            lax.fori_loop(queued, len(write_due), write_batch, None)

        pl.run_scoped(run, pltpu.SemaphoreType.DMA((n_chunks + 2,)))
        pltpu.make_async_copy(o_buf, o_hbm, out_sem.at[0]).wait()

    out = pl.pallas_call(
        kernel_function,
        in_specs=[pl.BlockSpec(memory_space=pl.ANY)] * 4,
        out_specs=pl.BlockSpec(memory_space=pl.ANY),
        out_shape=jax.ShapeDtypeStruct((n_pieces, S, C), dtype),
        scratch_shapes=[
            pltpu.VMEM((n_pieces, S, C), dtype),
            pltpu.VMEM((n_rows, W // 2, C), p_coarse.dtype),
            pltpu.VMEM((n_pieces, S, C), dtype),
            pltpu.VMEM((C, C), w_lat.dtype),
            pltpu.VMEM((C, C), w_out.dtype),
            pltpu.VMEM((C, C), dtype),
            pltpu.VMEM((n_tiles, G * W, _LANES), jnp.float32),
            pltpu.SemaphoreType.DMA((1,)),
        ],
        compiler_params=pltpu.CompilerParams(vmem_limit_bytes=124 * 2**20),
    )(
        c_fine.reshape(n_pieces, S, C),
        p_coarse.reshape(n_rows, W // 2, C),
        w_lat,
        w_out.reshape(C, C),
    )
    return out.reshape(B, H, W, C)
```

```python
import jax
import jax.numpy as jnp
from jax import lax
import jax.experimental.pallas as pl
import jax.experimental.pallas.tpu as pltpu

_LANES = 128
_STREAMS = 6
_PIECE = 32
_ROWS = 4
_READ_STEPS = 0.6
_LAST_READ = 3
_BATCH = 8
_BACKLOG = 40
_PACE = 22


@jax.jit
def pallas_standalone__detection_seg_fpn_lateral__vision_kernel(
    c_fine: jax.Array,
    p_coarse: jax.Array,
    w_lat: jax.Array,
    w_out: jax.Array,
):
    B, H, W, C = c_fine.shape
    dtype = c_fine.dtype
    A, S, G = _STREAMS, _PIECE, _ROWS
    n_rows = B * H // 2
    band = n_rows // A
    spare = n_rows - A * band
    ppr = 2 * W // S
    n_pieces = n_rows * ppr
    stream = n_pieces // A
    n_steps = n_rows // G
    n_tiles = C // _LANES
    assert w_out.shape == (1, 1, C, C) and p_coarse.shape == (B, H // 2, W // 2, C)
    assert n_rows % G == 0 and W % S == 0 and C % _LANES == 0
    assert 0 < spare < G and ppr % _BATCH == 0 and _LAST_READ < ppr

    order = list(range(A * band, n_rows))
    order += [a * band + i for i in range(band) for a in reversed(range(A))]
    step_of = {row: pos // G for pos, row in enumerate(order)}
    switch = int(_READ_STEPS * n_steps)

    lead = G - spare
    chunks = [(A - lead, lead, 0, 1), (0, A - lead, 0, 1)]
    i = 1
    while i < band:
        n = min(max(i // 2, 1), band - i)
        chunks.append((0, A, i, n))
        i += n
    n_chunks = len(chunks)
    read_due = [min([switch] + [step_of[b * band + i] for b in range(a, a + na)])
                for a, na, i, _ in chunks]
    last_read_due = min(step_of[b * band + band - 1] for b in range(A))

    def ready(k):
        return max(step_of[(a * stream + k) // ppr] for a in range(A)) + 1

    early = range(band * ppr, stream)
    assert all(ready(k) <= switch for k in early)
    assert all(step_of[k // ppr] < switch for k in range(A * stream, n_pieces))
    write_due = []
    for k in range(0, band * ppr, _BATCH):
        paced = switch + pl.cdiv(max(k + _BATCH - _BACKLOG, 0), _PACE)
        needs = [ready(k + b) for b in range(_BATCH)]
        write_due.append(max([min(paced, n_steps)] + needs + write_due[-1:]))

    def kernel_function(c_hbm, p_hbm, wl_hbm, wo_hbm, o_hbm,
                        c_buf, p_buf, o_buf, wl, wo, wf, up_buf, out_sem):
        def split(ref, n):
            return ref.at[pl.ds(0, A * n)].reshape(A, n, *ref.shape[1:])

        def copy(src, dst, idx, sem):
            return pltpu.make_async_copy(src.at[idx], dst.at[idx], sem)

        def write(k):
            copy(split(o_buf, stream), split(o_hbm, stream), (slice(None), k),
                 out_sem.at[0]).start()

        def write_batch(b, carry):
            for k in range(_BATCH):
                write(b * _BATCH + k)
            return carry

        def compute(step):
            rows = []
            for g in range(G):
                pos = step * G + g
                m = jnp.maximum(pos - spare, 0)
                banded = (A - 1 - lax.rem(m, A)) * band + lax.div(m, A)
                rows.append(jnp.where(pos < spare, A * band + pos, banded))
            p = jnp.concatenate([p_buf[r] for r in rows], axis=0)
            q = jnp.dot(p, wo[...], preferred_element_type=jnp.float32)
            for t in range(n_tiles):
                for e in range(2):
                    up_buf[t, pl.ds(e, G * W // 2, stride=2), :] = (
                        q[:, t * _LANES:(t + 1) * _LANES])
            up = jnp.concatenate([up_buf[t] for t in range(n_tiles)], axis=1)
            for j in range(2):
                idx = [pl.ds(r * ppr + j * (W // S), W // S) for r in rows]
                c = jnp.concatenate([c_buf[s].reshape(W, C) for s in idx], axis=0)
                lat = jnp.dot(c, wf[...], preferred_element_type=jnp.float32)
                res = (lat + up).astype(dtype)
                for g, s in enumerate(idx):
                    o_buf[s] = res[g * W:(g + 1) * W].reshape(W // S, S, C)

        def run(in_sem):
            def weights():
                return [pltpu.make_async_copy(wl_hbm, wl, in_sem.at[n_chunks]),
                        pltpu.make_async_copy(wo_hbm, wo, in_sem.at[n_chunks])]

            def reads(k):
                a, na, i, n = chunks[k]
                held = _LAST_READ if k == n_chunks - 1 else 0
                sem = in_sem.at[k]
                copies = [
                    copy(split(p_hbm, band), split(p_buf, band),
                         (pl.ds(a, na), pl.ds(i, n)), sem),
                    copy(split(c_hbm, band * ppr), split(c_buf, band * ppr),
                         (pl.ds(a, na), pl.ds(i * ppr, n * ppr - held)), sem),
                ]
                if k == 0:
                    copies += [
                        copy(p_hbm, p_buf, pl.ds(A * band, spare), sem),
                        copy(c_hbm, c_buf, pl.ds(A * band * ppr, spare * ppr), sem),
                    ]
                return copies

            def last_read():
                return copy(split(c_hbm, band * ppr), split(c_buf, band * ppr),
                            (slice(None), pl.ds(band * ppr - _LAST_READ, _LAST_READ)),
                            in_sem.at[n_chunks + 1])

            for x in weights():
                x.start()
            for k in range(n_chunks):
                for x in reads(k):
                    x.start()
            last_read().start()

            for x in weights():
                x.wait()
            wf[...] = jnp.dot(
                wl[...], wo[...], preferred_element_type=jnp.float32
            ).astype(wf.dtype)

            def body(step, queued):
                for k in range(n_chunks):
                    @pl.when(step == read_due[k])
                    def _(k=k):
                        for x in reads(k):
                            x.wait()

                @pl.when(step == switch)
                def _():
                    for k in early:
                        write(k)
                    if A * stream < n_pieces:
                        copy(o_buf, o_hbm, pl.ds(A * stream, n_pieces - A * stream),
                             out_sem.at[0]).start()

                target = queued
                for due in sorted(set(write_due) - {n_steps}):
                    count = sum(d <= due for d in write_due)
                    target = jnp.where(step == due, count, target)
                lax.fori_loop(queued, target, write_batch, None)

                @pl.when(step == last_read_due)
                def _():
                    last_read().wait()

                compute(step)
                return target

            queued = lax.fori_loop(0, n_steps, body, 0)
            lax.fori_loop(queued, len(write_due), write_batch, None)

        pl.run_scoped(run, pltpu.SemaphoreType.DMA((n_chunks + 2,)))
        pltpu.make_async_copy(o_buf, o_hbm, out_sem.at[0]).wait()

    out = pl.pallas_call(
        kernel_function,
        in_specs=[pl.BlockSpec(memory_space=pl.ANY)] * 4,
        out_specs=pl.BlockSpec(memory_space=pl.ANY),
        out_shape=jax.ShapeDtypeStruct((n_pieces, S, C), dtype),
        scratch_shapes=[
            pltpu.VMEM((n_pieces, S, C), dtype),
            pltpu.VMEM((n_rows, W // 2, C), p_coarse.dtype),
            pltpu.VMEM((n_pieces, S, C), dtype),
            pltpu.VMEM((C, C), w_lat.dtype),
            pltpu.VMEM((C, C), w_out.dtype),
            pltpu.VMEM((C, C), dtype),
            pltpu.VMEM((n_tiles, G * W, _LANES), jnp.float32),
            pltpu.SemaphoreType.DMA((1,)),
        ],
        compiler_params=pltpu.CompilerParams(vmem_limit_bytes=124 * 2**20),
    )(
        c_fine.reshape(n_pieces, S, C),
        p_coarse.reshape(n_rows, W // 2, C),
        w_lat,
        w_out.reshape(C, C),
    )
    return out.reshape(B, H, W, C)
```
